```python
import os as _os
_os.environ.setdefault("JAX_PLATFORMS", "cpu")
import jax
import jax.numpy as jnp

def _softmax(x, axis=-1):
    return jax.nn.softmax(x, axis=axis)
def _gelu(x):
    return jax.nn.gelu(x, approximate=True)
def _silu(x):
    return jax.nn.silu(x)
def _sigmoid(x):
    return jax.nn.sigmoid(x)
def _layernorm(x, axis=-1, eps=1e-5):
    m = jnp.mean(x, axis=axis, keepdims=True)
    v = jnp.var(x, axis=axis, keepdims=True)
    return (x - m) / jnp.sqrt(v + eps)
def _scatter_add(tgt, idx, src, axis=0):
    return tgt.at[idx].add(src)
def _segment_sum(src, seg, n):
    return jax.ops.segment_sum(src, seg, n)
class _Rng:
    def __init__(self, key):
        self._k = key
    def _next(self):
        self._k, sub = jax.random.split(self._k)
        return sub
    def normal(self, shape):
        return jax.random.normal(self._next(), shape, dtype=jnp.bfloat16)
    def randint(self, lo, hi, shape):
        return jax.random.randint(self._next(), shape, lo, hi, dtype=jnp.int32)
    def uniform(self, shape, lo=0.0, hi=1.0):
        return jax.random.uniform(self._next(), shape, jnp.bfloat16, lo, hi)
    def permutation(self, n):
        return jax.random.permutation(self._next(), n)


kernel_name = 'sequential_preLN__sliding_local_dilated__dense_activation_mish__prompt'

def setup_inputs():
    _rng = _Rng(jax.random.key(int.from_bytes(__import__("os").urandom(4), "little")))
    _w = (lambda a: (lambda t: t.astype(jnp.bfloat16) if jnp.issubdtype(t.dtype, jnp.floating) else t)(jnp.asarray(a)))
    def _A_setup():
        B, S, D = 1, 2048, 512
        return {
            "x": _w((lambda *s: _rng.normal(s) * 0.05)(B, S, D)),
            "wqkv": _w((lambda *s: _rng.normal(s) * 0.05)(D, 3 * D)),
            "wo": _w((lambda *s: _rng.normal(s) * 0.05)(D, D)),
        }
    _A_in = _A_setup()

    def _B_setup():
        B, S, D, F = 1, 2048, 512, 1376
        return {
            "x": _w((lambda *s: _rng.normal(s) * 0.05)(B, S, D)),
            "w1": _w((lambda *s: _rng.normal(s) * 1.6)(D, F) * (D ** -0.5)),
            "b1": _w((lambda *s: _rng.normal(s) * 0.1)(F)),
            "w2": _w((lambda *s: _rng.normal(s) * 0.1)(F, D) * (F ** -0.5)),
        }
    _B_in = _B_setup()

    return {
        "A_x": _A_in["x"],
        "A_wqkv": _A_in["wqkv"],
        "A_wo": _A_in["wo"],
        "B_x": _B_in["x"],
        "B_w1": _B_in["w1"],
        "B_b1": _B_in["b1"],
        "B_w2": _B_in["w2"],
    }

def reference(A_x, A_wqkv, A_wo, B_x, B_w1, B_b1, B_w2):
    def _A_ref(x, wqkv, wo):
        B, S, D = x.shape
        H = 32; Dh = D // H
        W, dil = 8, 2
        qkv = (lambda x, *d: x.transpose(*d))((x @ wqkv).reshape(B, S, 3, H, Dh), 2, 0, 3, 1, 4)
        q, k, v = qkv[0], qkv[1], qkv[2]
        scale = Dh ** -0.5
        pos = jnp.arange(S)
        off = jnp.arange(W) * dil
        idx = pos[:, None] - off[None, :]
        mask = idx >= 0
        idx_c = jnp.where(mask, idx, 0).reshape(-1)
        kg = k[:, :, idx_c, :].reshape(B, H, S, W, Dh)
        vg = v[:, :, idx_c, :].reshape(B, H, S, W, Dh)
        logits = jnp.einsum("bhsd,bhswd->bhsw", q, kg) * scale
        logits = jnp.where(mask[None, None, :, :], logits, -1e9)
        attn = _softmax(logits, axis=-1)
        o = jnp.einsum("bhsw,bhswd->bhsd", attn, vg)
        return (lambda x, *d: x.transpose(*d))(o, 0, 2, 1, 3).reshape(B, S, D) @ wo

    def _B_ref(x, w1, b1, w2):
        h = jnp.einsum("bsd,df->bsf", x, w1) + b1
        sp = jnp.log1p(jnp.exp(-jnp.abs(h))) + jnp.where(h > 0, h, jnp.zeros_like(h))
        act = h * jnp.tanh(sp)
        return jnp.einsum("bsf,fd->bsd", act, w2)

    x = A_x
    h = x + _A_ref(_layernorm(x, axis=-1), A_wqkv, A_wo)
    h2 = h + _B_ref(_layernorm(h, axis=-1), B_w1, B_b1, B_w2)
    return h2
```

```python
import functools

import jax
import jax.numpy as jnp
from jax import lax
from jax.experimental import pallas as pl
from jax.experimental.pallas import tpu as pltpu

_H = 32
_W = 8
_DIL = 2
_HALO = 16
_EPS = 1e-5


def _ln(x):
    m = jnp.mean(x, axis=-1, keepdims=True)
    xc = x - m
    v = jnp.mean(xc * xc, axis=-1, keepdims=True)
    return xc / jnp.sqrt(v + _EPS)


def _kernel(x_ref, wqkv_ref, wo_ref, w1_ref, b1_ref, w2_ref, o_ref,
            wqkv_p, wo_p, kbuf, vbuf, *, T, D):
    i = pl.program_id(0)
    Dh = D // _H
    f32 = jnp.float32
    bf16 = jnp.bfloat16

    @pl.when(i == 0)
    def _():
        r = lax.broadcasted_iota(jnp.int32, (D, D), 0)
        c = lax.broadcasted_iota(jnp.int32, (D, D), 1)
        P = (r == (c % _H) * Dh + c // _H).astype(bf16)
        for j in range(3):
            wqkv_p[:, j * D:(j + 1) * D] = jnp.dot(
                wqkv_ref[:, j * D:(j + 1) * D], P,
                preferred_element_type=f32).astype(bf16)
        PT = (c == (r % _H) * Dh + r // _H).astype(bf16)
        wo_p[...] = jnp.dot(PT, wo_ref[...],
                            preferred_element_type=f32).astype(bf16)
        kbuf[0:_HALO, :] = jnp.zeros((_HALO, D), f32)
        vbuf[0:_HALO, :] = jnp.zeros((_HALO, D), f32)

    x = x_ref[...].astype(f32)
    ln1 = _ln(x).astype(bf16)
    qkv = jnp.dot(ln1, wqkv_p[...], preferred_element_type=f32)
    q = qkv[:, 0:D] * (Dh ** -0.5)
    kbuf[_HALO:_HALO + T, :] = qkv[:, D:2 * D]
    vbuf[_HALO:_HALO + T, :] = qkv[:, 2 * D:3 * D]

    rows = i * T + lax.broadcasted_iota(jnp.int32, (T, 128), 0)
    nt = D // 128
    logits = []
    for w in range(_W):
        ks = kbuf[_HALO - _DIL * w:_HALO - _DIL * w + T, :]
        p = q * ks
        l = p[:, 0:128]
        for j in range(1, nt):
            l = l + p[:, j * 128:(j + 1) * 128]
        l = l + pltpu.roll(l, 64, 1)
        l = l + pltpu.roll(l, 32, 1)
        l = jnp.where(rows >= _DIL * w, l, -1e9)
        logits.append(l)
    m = logits[0]
    for w in range(1, _W):
        m = jnp.maximum(m, logits[w])
    es = [jnp.exp(l - m) for l in logits]
    den = es[0]
    for w in range(1, _W):
        den = den + es[w]
    inv = 1.0 / den
    o = None
    for w in range(_W):
        a = es[w] * inv
        a = jnp.concatenate([a] * nt, axis=1)
        vs = vbuf[_HALO - _DIL * w:_HALO - _DIL * w + T, :]
        o = a * vs if o is None else o + a * vs

    kbuf[0:_HALO, :] = kbuf[T:T + _HALO, :]
    vbuf[0:_HALO, :] = vbuf[T:T + _HALO, :]

    h = x + jnp.dot(o.astype(bf16), wo_p[...], preferred_element_type=f32)

    ln2 = _ln(h).astype(bf16)
    h1 = jnp.dot(ln2, w1_ref[...], preferred_element_type=f32) + b1_ref[...].astype(f32)
    sp = jnp.log1p(jnp.exp(-jnp.abs(h1))) + jnp.maximum(h1, 0.0)
    act = (h1 * jnp.tanh(sp)).astype(bf16)
    y = jnp.dot(act, w2_ref[...], preferred_element_type=f32)
    o_ref[...] = (h + y).astype(o_ref.dtype)


@jax.jit
def pallas_sequential_preLN__sliding_local_dilated__dense_activation_mish__prompt_kernel(
    A_x: jax.Array,
    A_wqkv: jax.Array,
    A_wo: jax.Array,
    B_x: jax.Array,
    B_w1: jax.Array,
    B_b1: jax.Array,
    B_w2: jax.Array,
):
    B, S, D = A_x.shape
    F = B_w1.shape[1]
    T = 256
    x2 = A_x.reshape(B * S, D)
    b1 = B_b1.reshape(1, F)

    const = lambda i: (0, 0)
    out = pl.pallas_call(
        functools.partial(_kernel, T=T, D=D),
        grid=(S // T,),
        in_specs=[
            pl.BlockSpec((T, D), lambda i: (i, 0)),
            pl.BlockSpec((D, 3 * D), const),
            pl.BlockSpec((D, D), const),
            pl.BlockSpec((D, F), const),
            pl.BlockSpec((1, F), const),
            pl.BlockSpec((F, D), const),
        ],
        out_specs=pl.BlockSpec((T, D), lambda i: (i, 0)),
        out_shape=jax.ShapeDtypeStruct((B * S, D), A_x.dtype),
        scratch_shapes=[
            pltpu.VMEM((D, 3 * D), jnp.bfloat16),
            pltpu.VMEM((D, D), jnp.bfloat16),
            pltpu.VMEM((T + _HALO, D), jnp.float32),
            pltpu.VMEM((T + _HALO, D), jnp.float32),
        ],
        compiler_params=pltpu.CompilerParams(
            dimension_semantics=("arbitrary",),
            vmem_limit_bytes=96 * 1024 * 1024,
        ),
    )(x2, A_wqkv, A_wo, B_w1, b1, B_w2)
    return out.reshape(B, S, D)
```

```python
import functools

import jax
import jax.numpy as jnp
from jax import lax
from jax.experimental import pallas as pl
from jax.experimental.pallas import tpu as pltpu

_H = 32
_W = 8
_DIL = 2
_HALO = 16
_EPS = 1e-5
_T = 256
_RC = 32
_FC = 256


def _ln(x):
    m = jnp.mean(x, axis=-1, keepdims=True)
    xc = x - m
    v = jnp.mean(xc * xc, axis=-1, keepdims=True)
    return xc / jnp.sqrt(v + _EPS)


def _interleave(main, side):
    nm, ns = len(main), len(side)
    k = 0
    for j, piece in enumerate(main):
        piece()
        while k < ns and k * nm < (j + 1) * ns:
            side[k]()
            k += 1
    while k < ns:
        side[k]()
        k += 1


def _kernel(x_hbm, wqkv_hbm, wo_hbm, w1t_hbm, b1_ref, w2_hbm, o_hbm,
            xbuf, wqkv_raw, wo_raw, w1t, w2, wqkv_p, wo_p, wo_f, qbuf, kbuf, vbuf, abuf, obuf,
            sem_in, sem_out, *, T, S, D, F):
    n = S // T
    Dh = D // _H
    nt = D // 128
    f32 = jnp.float32
    bf16 = jnp.bfloat16

    cp_x0 = pltpu.make_async_copy(x_hbm.at[0:T], xbuf.at[0:T], sem_in.at[0])
    cp_wqkv = [pltpu.make_async_copy(wqkv_hbm.at[:, j * D:(j + 1) * D],
                                     wqkv_raw.at[:, j * D:(j + 1) * D], sem_in.at[6 + j])
               for j in range(3)]
    cp_x1 = pltpu.make_async_copy(x_hbm.at[T:2 * T], xbuf.at[T:2 * T], sem_in.at[2])
    cp_xr = pltpu.make_async_copy(x_hbm.at[2 * T:S], xbuf.at[2 * T:S], sem_in.at[1])
    cp_wo = pltpu.make_async_copy(wo_hbm, wo_raw, sem_in.at[3])
    cp_w1 = pltpu.make_async_copy(w1t_hbm, w1t, sem_in.at[4])
    cp_w2 = pltpu.make_async_copy(w2_hbm, w2, sem_in.at[5])
    for cp in (cp_wqkv[0], cp_x0, cp_wqkv[1], cp_x1, cp_wqkv[2], cp_wo, cp_w1, cp_w2, cp_xr):
        cp.start()

    r = lax.broadcasted_iota(jnp.int32, (D, D), 0)
    c = lax.broadcasted_iota(jnp.int32, (D, D), 1)
    P = (r == (c % _H) * Dh + c // _H).astype(bf16)
    def perm(j):
        pj = jnp.dot(wqkv_raw[:, j * D:(j + 1) * D], P, preferred_element_type=f32)
        if j == 0:
            pj = pj * (Dh ** -0.5)
        wqkv_p[:, j * D:(j + 1) * D] = pj.astype(bf16)

    kbuf[1, T:T + _HALO, :] = jnp.zeros((_HALO, D), f32)
    vbuf[1, T:T + _HALO, :] = jnp.zeros((_HALO, D), f32)

    def pieces_a(t, slot):
        st = {}

        def p_ln():
            x = xbuf[pl.ds(pl.multiple_of(t * T, T), T), :].astype(f32)
            st['ln1'] = _ln(x).astype(bf16)

        def p_q():
            qbuf[slot] = jnp.dot(st['ln1'], wqkv_p[:, 0:D],
                                 preferred_element_type=f32)

        def p_k():
            kbuf[slot, _HALO:_HALO + T, :] = jnp.dot(
                st['ln1'], wqkv_p[:, D:2 * D], preferred_element_type=f32)
            kbuf[slot, 0:_HALO, :] = kbuf[1 - slot, T:T + _HALO, :]

        def p_v():
            vbuf[slot, _HALO:_HALO + T, :] = jnp.dot(
                st['ln1'], wqkv_p[:, 2 * D:3 * D], preferred_element_type=f32)
            vbuf[slot, 0:_HALO, :] = vbuf[1 - slot, T:T + _HALO, :]

        return [p_ln, p_q, p_k, p_v]

    def pieces_b(t, slot):
        def chunk(r0):
            R = _RC
            q = qbuf[slot, r0:r0 + R, :]
            rows = t * T + r0 + lax.broadcasted_iota(jnp.int32, (R, 128), 0)
            logits = []
            for w in range(_W):
                b = _HALO - _DIL * w + r0
                p = q * kbuf[slot, b:b + R, :]
                l = p[:, 0:128]
                for j in range(1, nt):
                    l = l + p[:, j * 128:(j + 1) * 128]
                l = l + pltpu.roll(l, 64, 1)
                l = l + pltpu.roll(l, 32, 1)
                logits.append(jnp.where(rows >= _DIL * w, l, -1e9))
            m = logits[0]
            for w in range(1, _W):
                m = jnp.maximum(m, logits[w])
            es = [jnp.exp(l - m) for l in logits]
            den = es[0]
            for w in range(1, _W):
                den = den + es[w]
            inv = 1.0 / den
            o = None
            for w in range(_W):
                b = _HALO - _DIL * w + r0
                a = jnp.concatenate([es[w] * inv] * nt, axis=1)
                vs = vbuf[slot, b:b + R, :]
                o = a * vs if o is None else o + a * vs
            abuf[slot, r0:r0 + R, :] = o.astype(bf16)
        return [functools.partial(chunk, r0) for r0 in range(0, T, _RC)]

    def pieces_c(t, slot):
        st = {}
        row0 = pl.multiple_of(t * T, T)

        def p_wo():
            x = xbuf[pl.ds(row0, T), :].astype(f32)
            h = x + jnp.dot(abuf[slot], wo_p[...], preferred_element_type=f32)
            st['h'] = h
            st['ln2'] = _ln(h).astype(bf16)
            st['y'] = h

        def p_f(f0, f1):
            h1 = lax.dot_general(st['ln2'], w1t[f0:f1, :], (((1,), (1,)), ((), ())),
                                 preferred_element_type=f32) + b1_ref[:, f0:f1].astype(f32)
            sp = jnp.log1p(jnp.exp(-jnp.abs(h1))) + jnp.maximum(h1, 0.0)
            act = (h1 * jnp.tanh(sp)).astype(bf16)
            st['y'] = st['y'] + jnp.dot(act, w2[f0:f1, :], preferred_element_type=f32)

        def p_out():
            obuf[pl.ds(row0, T), :] = st['y'].astype(obuf.dtype)
            pltpu.make_async_copy(obuf.at[pl.ds(row0, T)], o_hbm.at[pl.ds(row0, T)],
                                  sem_out.at[t]).start()

        fs = [(f0, min(f0 + _FC, F)) for f0 in range(0, F, _FC)]
        return [p_wo] + [functools.partial(p_f, a, b) for a, b in fs] + [p_out]

    def run(pieces):
        for p in pieces:
            p()

    a0 = pieces_a(0, 0)
    a1 = pieces_a(1, 1)
    cp_wqkv[0].wait()
    cp_x0.wait()
    perm(0)
    a0[0]()
    cp_wqkv[1].wait()
    cp_x1.wait()
    perm(1)
    a1[0]()
    a0[1]()
    cp_wqkv[2].wait()
    cp_wo.wait()
    perm(2)
    for j in range(nt):
        wo_f[j] = wo_raw[:, j * 128:(j + 1) * 128].astype(f32)
    for j in range(nt):
        for d in range(Dh):
            wo_p[d * _H:(d + 1) * _H, j * 128:(j + 1) * 128] = (
                wo_f[j, pl.ds(d, _H, stride=Dh), :].astype(bf16))
    a0[2]()
    a0[3]()
    _interleave(a1[1:], pieces_b(0, 0))
    cp_w1.wait()
    cp_w2.wait()
    cp_xr.wait()

    def body(i, carry):
        slot = i % 2
        main = pieces_c(i, slot) + pieces_a(i + 2, slot)
        _interleave(main, pieces_b(i + 1, 1 - slot))
        return carry

    lax.fori_loop(0, n - 2, body, 0)
    _interleave(pieces_c(n - 2, (n - 2) % 2), pieces_b(n - 1, (n - 1) % 2))
    run(pieces_c(n - 1, (n - 1) % 2))
    for t in range(n):
        pltpu.make_async_copy(obuf.at[t * T:(t + 1) * T], o_hbm.at[t * T:(t + 1) * T],
                              sem_out.at[t]).wait()


@jax.jit
def pallas_sequential_preLN__sliding_local_dilated__dense_activation_mish__prompt_kernel(
    A_x, A_wqkv, A_wo, B_x, B_w1, B_b1, B_w2,
):
    B, S, D = A_x.shape
    F = B_w1.shape[1]
    T = _T
    n = S // T
    x2 = A_x.reshape(B * S, D)
    b1 = B_b1.reshape(1, F)
    bf16 = jnp.bfloat16
    f32 = jnp.float32
    anyspec = pl.BlockSpec(memory_space=pl.ANY)
    out = pl.pallas_call(
        functools.partial(_kernel, T=T, S=S, D=D, F=F),
        in_specs=[anyspec, anyspec, anyspec, anyspec,
                  pl.BlockSpec(memory_space=pltpu.VMEM), anyspec],
        out_specs=anyspec,
        out_shape=jax.ShapeDtypeStruct((B * S, D), A_x.dtype),
        scratch_shapes=[
            pltpu.VMEM((S, D), bf16),
            pltpu.VMEM((D, 3 * D), bf16),
            pltpu.VMEM((D, D), bf16),
            pltpu.VMEM((F, D), bf16),
            pltpu.VMEM((F, D), bf16),
            pltpu.VMEM((D, 3 * D), bf16),
            pltpu.VMEM((D, D), bf16),
            pltpu.VMEM((D // 128, D, 128), f32),
            pltpu.VMEM((2, T, D), f32),
            pltpu.VMEM((2, T + _HALO, D), f32),
            pltpu.VMEM((2, T + _HALO, D), f32),
            pltpu.VMEM((2, T, D), bf16),
            pltpu.VMEM((S, D), bf16),
            pltpu.SemaphoreType.DMA((9,)),
            pltpu.SemaphoreType.DMA((n,)),
        ],
        compiler_params=pltpu.CompilerParams(
            vmem_limit_bytes=127 * 1024 * 1024,
        ),
    )(x2, A_wqkv, A_wo, B_w1.T, b1, B_w2)
    return out.reshape(B, S, D)
```

```python
import functools

import jax
import jax.numpy as jnp
from jax import lax
from jax.experimental import pallas as pl
from jax.experimental.pallas import tpu as pltpu

_H = 32
_W = 8
_DIL = 2
_HALO = 16
_EPS = 1e-5
_T = 256
_RC = 32
_FC = 256


def _ln(x):
    m = jnp.mean(x, axis=-1, keepdims=True)
    xc = x - m
    v = jnp.mean(xc * xc, axis=-1, keepdims=True)
    return xc / jnp.sqrt(v + _EPS)


def _interleave(main, side):
    nm, ns = len(main), len(side)
    k = 0
    for j, piece in enumerate(main):
        piece()
        while k < ns and k * nm < (j + 1) * ns:
            side[k]()
            k += 1
    while k < ns:
        side[k]()
        k += 1


def _kernel(x_hbm, wqkv_hbm, wo_hbm, w1t_hbm, b1_ref, w2_hbm, o_hbm,
            xbuf, wqkv_raw, wo_raw, w1t, w2, wqkv_p, wo_p, wo_f, qbuf, kbuf, vbuf, abuf, obuf,
            sem_in, sem_out, *, T, S, D, F):
    n = S // T
    Dh = D // _H
    nt = D // 128
    f32 = jnp.float32
    bf16 = jnp.bfloat16

    cp_x0 = pltpu.make_async_copy(x_hbm.at[0:T], xbuf.at[0:T], sem_in.at[0])
    cp_wqkv = [pltpu.make_async_copy(wqkv_hbm.at[:, j * D:(j + 1) * D],
                                     wqkv_raw.at[:, j * D:(j + 1) * D], sem_in.at[6 + j])
               for j in range(3)]
    cp_x1 = pltpu.make_async_copy(x_hbm.at[T:2 * T], xbuf.at[T:2 * T], sem_in.at[2])
    cp_xr = pltpu.make_async_copy(x_hbm.at[2 * T:S], xbuf.at[2 * T:S], sem_in.at[1])
    cp_wo = pltpu.make_async_copy(wo_hbm, wo_raw, sem_in.at[3])
    cp_w1 = pltpu.make_async_copy(w1t_hbm, w1t, sem_in.at[4])
    cp_w2 = pltpu.make_async_copy(w2_hbm, w2, sem_in.at[5])
    for cp in (cp_wqkv[0], cp_x0, cp_wqkv[1], cp_x1, cp_wqkv[2], cp_wo, cp_w1, cp_w2, cp_xr):
        cp.start()

    r = lax.broadcasted_iota(jnp.int32, (D, D), 0)
    c = lax.broadcasted_iota(jnp.int32, (D, D), 1)
    P = (r == (c % _H) * Dh + c // _H).astype(bf16)
    def perm(j):
        pj = jnp.dot(wqkv_raw[:, j * D:(j + 1) * D], P, preferred_element_type=f32)
        if j == 0:
            pj = pj * (Dh ** -0.5)
        wqkv_p[:, j * D:(j + 1) * D] = pj.astype(bf16)

    kbuf[1, T:T + _HALO, :] = jnp.zeros((_HALO, D), f32)
    vbuf[1, T:T + _HALO, :] = jnp.zeros((_HALO, D), f32)

    def pieces_a(t, slot):
        st = {}

        def p_ln():
            x = xbuf[pl.ds(pl.multiple_of(t * T, T), T), :].astype(f32)
            st['ln1'] = _ln(x).astype(bf16)

        def p_q():
            qbuf[slot] = jnp.dot(st['ln1'], wqkv_p[:, 0:D],
                                 preferred_element_type=f32)

        def p_k():
            kbuf[slot, _HALO:_HALO + T, :] = jnp.dot(
                st['ln1'], wqkv_p[:, D:2 * D], preferred_element_type=f32)
            kbuf[slot, 0:_HALO, :] = kbuf[1 - slot, T:T + _HALO, :]

        def p_v():
            vbuf[slot, _HALO:_HALO + T, :] = jnp.dot(
                st['ln1'], wqkv_p[:, 2 * D:3 * D], preferred_element_type=f32)
            vbuf[slot, 0:_HALO, :] = vbuf[1 - slot, T:T + _HALO, :]

        return [p_ln, p_q, p_k, p_v]

    def pieces_b(t, slot):
        def chunk(r0):
            R = _RC
            q = qbuf[slot, r0:r0 + R, :]
            rows = t * T + r0 + lax.broadcasted_iota(jnp.int32, (R, 128), 0)
            logits = []
            for w in range(_W):
                b = _HALO - _DIL * w + r0
                p = q * kbuf[slot, b:b + R, :]
                l = p[:, 0:128]
                for j in range(1, nt):
                    l = l + p[:, j * 128:(j + 1) * 128]
                l = l + pltpu.roll(l, 64, 1)
                l = l + pltpu.roll(l, 32, 1)
                logits.append(jnp.where(rows >= _DIL * w, l, -1e9))
            m = logits[0]
            for w in range(1, _W):
                m = jnp.maximum(m, logits[w])
            es = [jnp.exp(l - m) for l in logits]
            den = es[0]
            for w in range(1, _W):
                den = den + es[w]
            inv = 1.0 / den
            o = None
            for w in range(_W):
                b = _HALO - _DIL * w + r0
                a = jnp.concatenate([es[w]] * nt, axis=1)
                vs = vbuf[slot, b:b + R, :]
                o = a * vs if o is None else o + a * vs
            abuf[slot, r0:r0 + R, :] = (o * jnp.concatenate([inv] * nt, axis=1)).astype(bf16)
        return [functools.partial(chunk, r0) for r0 in range(0, T, _RC)]

    def pieces_c(t, slot):
        st = {}
        row0 = pl.multiple_of(t * T, T)

        def p_wo():
            x = xbuf[pl.ds(row0, T), :].astype(f32)
            h = x + jnp.dot(abuf[slot], wo_p[...], preferred_element_type=f32)
            st['h'] = h
            st['ln2'] = _ln(h).astype(bf16)
            st['y'] = h

        def p_f(f0, f1):
            h1 = lax.dot_general(st['ln2'], w1t[f0:f1, :], (((1,), (1,)), ((), ())),
                                 preferred_element_type=f32) + b1_ref[:, f0:f1].astype(f32)
            sp = jnp.log1p(jnp.exp(-jnp.abs(h1))) + jnp.maximum(h1, 0.0)
            act = (h1 * jnp.tanh(sp)).astype(bf16)
            st['y'] = st['y'] + jnp.dot(act, w2[f0:f1, :], preferred_element_type=f32)

        def p_out():
            obuf[pl.ds(row0, T), :] = st['y'].astype(obuf.dtype)
            pltpu.make_async_copy(obuf.at[pl.ds(row0, T)], o_hbm.at[pl.ds(row0, T)],
                                  sem_out.at[t]).start()

        fs = [(f0, min(f0 + _FC, F)) for f0 in range(0, F, _FC)]
        return [p_wo] + [functools.partial(p_f, a, b) for a, b in fs] + [p_out]

    def run(pieces):
        for p in pieces:
            p()

    a0 = pieces_a(0, 0)
    a1 = pieces_a(1, 1)
    cp_wqkv[0].wait()
    cp_x0.wait()
    perm(0)
    a0[0]()
    cp_wqkv[1].wait()
    cp_x1.wait()
    perm(1)
    a1[0]()
    a0[1]()
    cp_wqkv[2].wait()
    cp_wo.wait()
    perm(2)
    for j in range(nt):
        wo_f[j] = wo_raw[:, j * 128:(j + 1) * 128].astype(f32)
    for j in range(nt):
        for d in range(Dh):
            wo_p[d * _H:(d + 1) * _H, j * 128:(j + 1) * 128] = (
                wo_f[j, pl.ds(d, _H, stride=Dh), :].astype(bf16))
    a0[2]()
    a0[3]()
    _interleave(a1[1:], pieces_b(0, 0))
    cp_w1.wait()
    cp_w2.wait()
    cp_xr.wait()

    def body(i, carry):
        slot = i % 2
        main = pieces_c(i, slot) + pieces_a(i + 2, slot)
        _interleave(main, pieces_b(i + 1, 1 - slot))
        return carry

    lax.fori_loop(0, n - 2, body, 0)
    _interleave(pieces_c(n - 2, (n - 2) % 2), pieces_b(n - 1, (n - 1) % 2))
    run(pieces_c(n - 1, (n - 1) % 2))
    for t in range(n):
        pltpu.make_async_copy(obuf.at[t * T:(t + 1) * T], o_hbm.at[t * T:(t + 1) * T],
                              sem_out.at[t]).wait()


@jax.jit
def pallas_sequential_preLN__sliding_local_dilated__dense_activation_mish__prompt_kernel(
    A_x: jax.Array,
    A_wqkv: jax.Array,
    A_wo: jax.Array,
    B_x: jax.Array,
    B_w1: jax.Array,
    B_b1: jax.Array,
    B_w2: jax.Array,
):
    del B_x
    B, S, D = A_x.shape
    F = B_w1.shape[1]
    T = _T
    n = S // T
    x2 = A_x.reshape(B * S, D)
    b1 = B_b1.reshape(1, F)
    bf16 = jnp.bfloat16
    f32 = jnp.float32
    anyspec = pl.BlockSpec(memory_space=pl.ANY)
    out = pl.pallas_call(
        functools.partial(_kernel, T=T, S=S, D=D, F=F),
        in_specs=[anyspec, anyspec, anyspec, anyspec,
                  pl.BlockSpec(memory_space=pltpu.VMEM), anyspec],
        out_specs=anyspec,
        out_shape=jax.ShapeDtypeStruct((B * S, D), A_x.dtype),
        scratch_shapes=[
            pltpu.VMEM((S, D), bf16),
            pltpu.VMEM((D, 3 * D), bf16),
            pltpu.VMEM((D, D), bf16),
            pltpu.VMEM((F, D), bf16),
            pltpu.VMEM((F, D), bf16),
            pltpu.VMEM((D, 3 * D), bf16),
            pltpu.VMEM((D, D), bf16),
            pltpu.VMEM((D // 128, D, 128), f32),
            pltpu.VMEM((2, T, D), f32),
            pltpu.VMEM((2, T + _HALO, D), f32),
            pltpu.VMEM((2, T + _HALO, D), f32),
            pltpu.VMEM((2, T, D), bf16),
            pltpu.VMEM((S, D), bf16),
            pltpu.SemaphoreType.DMA((9,)),
            pltpu.SemaphoreType.DMA((n,)),
        ],
        compiler_params=pltpu.CompilerParams(
            vmem_limit_bytes=127 * 1024 * 1024,
        ),
    )(x2, A_wqkv, A_wo, B_w1.T, b1, B_w2)
    return out.reshape(B, S, D)
```
